```python
import jax
import jax.numpy as jnp

def _softmax(x, axis=-1):
    return jax.nn.softmax(x, axis=axis)

def _gelu(x):
    return jax.nn.gelu(x, approximate=True)

def _silu(x):
    return jax.nn.silu(x)

def _sigmoid(x):
    return jax.nn.sigmoid(x)

def _layernorm(x, axis=-1, eps=1e-05):
    m = jnp.mean(x, axis=axis, keepdims=True)
    v = jnp.var(x, axis=axis, keepdims=True)
    return (x - m) / jnp.sqrt(v + eps)

def _scatter_add(tgt, idx, src, axis=0):
    return tgt.at[idx].add(src)

def _segment_sum(src, seg, n):
    return jax.ops.segment_sum(src, seg, n)

class _Rng:

    def __init__(self, key):
        self._k = key

    def _next(self):
        self._k, sub = jax.random.split(self._k)
        return sub

    def normal(self, shape):
        return jax.random.normal(self._next(), shape, dtype=jnp.bfloat16)

    def randint(self, lo, hi, shape):
        return jax.random.randint(self._next(), shape, lo, hi, dtype=jnp.int32)

    def uniform(self, shape, lo=0.0, hi=1.0):
        return jax.random.uniform(self._next(), shape, jnp.bfloat16, lo, hi)

    def permutation(self, n):
        return jax.random.permutation(self._next(), n)
kernel_name = 'adaLN_cond__sliding_block_cached__dense_activation_gelu__decode'

def setup_inputs():
    _rng = _Rng(jax.random.key(int.from_bytes(__import__("os").urandom(4), "little")))
    _w = lambda a: (lambda t: t.astype(jnp.bfloat16) if jnp.issubdtype(t.dtype, jnp.floating) else t)(jnp.asarray(a))

    def _A_setup():
        B, Sq, D = (4, 1, 640)
        Hq, Hkv, Sk, Dh = (32, 32, 8192, 128)
        assert Hq % Hkv == 0, (Hq, Hkv)
        return {'x': _w((lambda *s: _rng.normal(s) * 0.05)(B, Sq, D)), 'k_cache': _w((lambda *s: _rng.normal(s) * 0.05)(B, Hkv, Sk, Dh)), 'v_cache': _w((lambda *s: _rng.normal(s) * 0.05)(B, Hkv, Sk, Dh)), 'wq': _w((lambda *s: _rng.normal(s) * 0.05)(D, Hq * Dh) * D ** (-0.5)), 'wo': _w((lambda *s: _rng.normal(s) * 0.05)(Hq * Dh, D) * (Hq * Dh) ** (-0.5))}
    _A_in = _A_setup()

    def _B_setup():
        B, S, D, F = (4, 1, 640, 1728)
        return {'x': _w((lambda *s: _rng.normal(s) * 0.05)(B, S, D)), 'w1': _w((lambda *s: _rng.normal(s) * 0.05)(D, F) * D ** (-0.5)), 'b1': _w((lambda *s: _rng.normal(s) * 0.05)(F) * 0.01), 'w2': _w((lambda *s: _rng.normal(s) * 0.05)(F, D) * F ** (-0.5)), 'b2': _w((lambda *s: _rng.normal(s) * 0.05)(D) * 0.01)}
    _B_in = _B_setup()
    return {'A_x': _A_in['x'], 'A_k_cache': _A_in['k_cache'], 'A_v_cache': _A_in['v_cache'], 'A_wq': _A_in['wq'], 'A_wo': _A_in['wo'], 'B_x': _B_in['x'], 'B_w1': _B_in['w1'], 'B_b1': _B_in['b1'], 'B_w2': _B_in['w2'], 'B_b2': _B_in['b2'], 'c': _w((lambda *s: _rng.normal(s) * 0.05)(4, 640)), 'w_mod': _w((lambda *s: _rng.normal(s) * 0.05)(640, 6 * 640) * 640 ** (-0.5))}

def reference(A_x, A_k_cache, A_v_cache, A_wq, A_wo, B_x, B_w1, B_b1, B_w2, B_b2, c, w_mod):

    def _A_ref(x, k_cache, v_cache, wq, wo):
        B, Sq, D = x.shape
        Hq, Dh = (32, 128)
        Hkv, Sk = (k_cache.shape[1], k_cache.shape[2])
        W = min(4096, max(256, Sk // 4))
        rep = Hq // Hkv
        q = (lambda x, *d: x.transpose(*d))((x @ wq).reshape(B, Sq, Hq, Dh), 0, 2, 1, 3)
        k = jnp.repeat(k_cache[:, :, Sk - W:, :], rep, axis=1)
        v = jnp.repeat(v_cache[:, :, Sk - W:, :], rep, axis=1)
        scores = jnp.einsum('bhqd,bhkd->bhqk', q, k) * Dh ** (-0.5)
        p = _softmax(scores, axis=-1)
        o = jnp.einsum('bhqk,bhkd->bhqd', p, v)
        return (lambda x, *d: x.transpose(*d))(o, 0, 2, 1, 3).reshape(B, Sq, Hq * Dh) @ wo

    def _B_ref(x, w1, b1, w2, b2):
        h = jnp.einsum('bsd,df->bsf', x, w1) + b1
        h = _gelu(h)
        return jnp.einsum('bsf,fd->bsd', h, w2) + b2
    x = A_x
    mod = (_silu(c) @ w_mod).reshape(c.shape[0], 6, 1, -1)
    sa, ca, ga, sb, cb, gb = (mod[:, 0].copy(), mod[:, 1].copy(), mod[:, 2].copy(), mod[:, 3].copy(), mod[:, 4].copy(), mod[:, 5].copy())
    h = _layernorm(x, axis=-1) * (1 + ca) + sa
    x = x + ga * _A_ref(h, A_k_cache, A_v_cache, A_wq, A_wo)
    h = _layernorm(x, axis=-1) * (1 + cb) + sb
    x = x + gb * _B_ref(h, B_w1, B_b1, B_w2, B_b2)
    return x
```

```python
import functools
import jax
import jax.numpy as jnp
from jax import lax
from jax.experimental import pallas as pl
from jax.experimental.pallas import tpu as pltpu

NBUF = 4
_NT = (((1,), (1,)), ((), ()))


def _layernorm(x, eps=1e-5):
    m = jnp.mean(x, axis=-1, keepdims=True)
    d = x - m
    v = jnp.mean(d * d, axis=-1, keepdims=True)
    return d / jnp.sqrt(v + eps)


def _kernel(x_hbm, k_hbm, v_hbm, wq_hbm, wo_hbm, w1t_hbm, b1_hbm, w2_hbm, b2_hbm, c_hbm, wm_hbm,
            out_ref,
            x_v, c_v, b1_v, b2_v, wm_v, wq_v, wo_v, w1t_v, w2_v, kbuf, vbuf, q_s, o_s, sem_w, sem_kv):
    B, H, SK, DH = k_hbm.shape
    W = kbuf.shape[2]
    D = x_v.shape[1]
    f32, bf16 = jnp.float32, jnp.bfloat16

    cp = pltpu.make_async_copy
    c_cp = cp(c_hbm, c_v, sem_w.at[0])
    x_cp = cp(x_hbm, x_v, sem_w.at[1])
    wma_cp = cp(wm_hbm.at[:, pl.ds(0, 2 * D)], wm_v.at[:, pl.ds(0, 2 * D)], sem_w.at[2])
    wq_cp = cp(wq_hbm, wq_v, sem_w.at[3])
    wo_cp = cp(wo_hbm, wo_v, sem_w.at[4])
    wmb_cp = cp(wm_hbm.at[:, pl.ds(2 * D, 4 * D)], wm_v.at[:, pl.ds(2 * D, 4 * D)], sem_w.at[5])
    b1_cp = cp(b1_hbm, b1_v, sem_w.at[6])
    b2_cp = cp(b2_hbm, b2_v, sem_w.at[7])
    w1_cp = cp(w1t_hbm, w1t_v, sem_w.at[8])
    w2_cp = cp(w2_hbm, w2_v, sem_w.at[9])

    def kv_cps(h, slot):
        return [cp(k_hbm.at[:, h, pl.ds(SK - W, W), :], kbuf.at[slot], sem_kv.at[slot, 0]),
                cp(v_hbm.at[:, h, pl.ds(SK - W, W), :], vbuf.at[slot], sem_kv.at[slot, 1])]

    for c_ in (c_cp, x_cp, wma_cp, wq_cp):
        c_.start()
    for i in range(NBUF):
        for c_ in kv_cps(i, i):
            c_.start()

    c_cp.wait()
    x_cp.wait()
    cc = c_v[...].astype(f32)
    sc = (cc * jax.nn.sigmoid(cc)).astype(bf16)
    x = x_v[...].astype(f32)
    ln = _layernorm(x)
    wma_cp.wait()
    moda = jnp.dot(sc, wm_v[:, 0:2 * D], preferred_element_type=f32)
    h = (ln * (1.0 + moda[:, D:2 * D]) + moda[:, 0:D]).astype(bf16)
    wq_cp.wait()
    q = jnp.dot(h, wq_v[...], preferred_element_type=f32)
    for hh in range(H):
        q_s[hh] = q[:, hh * DH:(hh + 1) * DH]

    scale = DH ** -0.5
    row = lax.broadcasted_iota(jnp.int32, (B, DH), 0)

    def body(hh, carry):
        slot = hh % NBUF
        kc, vc = kv_cps(hh, slot)
        qh = q_s[hh].astype(bf16)
        kc.wait()
        ps, ls = [], []
        for b in range(B):
            s = lax.dot_general(qh, kbuf[slot, b], _NT, preferred_element_type=f32) * scale
            m = jnp.max(s, axis=-1, keepdims=True)
            p = jnp.exp(s - m)
            ls.append(jnp.sum(p, axis=-1, keepdims=True))
            ps.append(p.astype(bf16))
        vc.wait()
        o = jnp.zeros((B, DH), f32)
        for b in range(B):
            ob = jnp.dot(ps[b], vbuf[slot, b], preferred_element_type=f32) / ls[b]
            o = jnp.where(row == b, ob, o)
        o_s[hh] = o

        @pl.when(hh + NBUF < H)
        def _():
            for c_ in kv_cps(hh + NBUF, slot):
                c_.start()

        @pl.when(hh + NBUF == H)
        def _():
            for c_ in (wo_cp, wmb_cp, b1_cp, b2_cp, w1_cp, w2_cp):
                c_.start()
        return carry

    lax.fori_loop(0, H, body, 0)

    o_all = jnp.concatenate([o_s[hh] for hh in range(H)], axis=-1).astype(bf16)
    wo_cp.wait()
    a = jnp.dot(o_all, wo_v[...], preferred_element_type=f32)
    wmb_cp.wait()
    modb = jnp.dot(sc, wm_v[:, 2 * D:6 * D], preferred_element_type=f32)
    x1 = x + modb[:, 0:D] * a
    h2 = (_layernorm(x1) * (1.0 + modb[:, 2 * D:3 * D]) + modb[:, D:2 * D]).astype(bf16)
    b1_cp.wait()
    b2_cp.wait()
    w1_cp.wait()
    u = lax.dot_general(h2, w1t_v[...], _NT, preferred_element_type=f32) + b1_v[...].astype(f32)[None, :]
    g = jax.nn.gelu(u, approximate=True).astype(bf16)
    w2_cp.wait()
    y = jnp.dot(g, w2_v[...], preferred_element_type=f32) + b2_v[...].astype(f32)[None, :]
    out_ref[...] = (x1 + modb[:, 3 * D:4 * D] * y).astype(out_ref.dtype)


@jax.jit
def pallas_adaLN_cond__sliding_block_cached__dense_activation_gelu__decode_kernel(A_x, A_k_cache, A_v_cache, A_wq, A_wo, B_x, B_w1, B_b1, B_w2, B_b2, c, w_mod):
    del B_x
    B, Sq, D = A_x.shape
    _, H, SK, DH = A_k_cache.shape
    W = min(4096, max(256, SK // 4))
    F = B_w1.shape[1]
    bf16 = jnp.bfloat16
    hbm = pl.BlockSpec(memory_space=pltpu.HBM)
    out = pl.pallas_call(
        _kernel,
        in_specs=[hbm] * 11,
        out_specs=pl.BlockSpec(memory_space=pltpu.VMEM),
        out_shape=jax.ShapeDtypeStruct((B, D), A_x.dtype),
        scratch_shapes=[
            pltpu.VMEM((B, D), bf16), pltpu.VMEM((B, D), bf16),
            pltpu.VMEM((F,), bf16), pltpu.VMEM((D,), bf16),
            pltpu.VMEM((D, 6 * D), bf16), pltpu.VMEM((D, H * DH), bf16), pltpu.VMEM((H * DH, D), bf16),
            pltpu.VMEM((F, D), bf16), pltpu.VMEM((F, D), bf16),
            pltpu.VMEM((NBUF, B, W, DH), bf16), pltpu.VMEM((NBUF, B, W, DH), bf16),
            pltpu.VMEM((H, B, DH), jnp.float32), pltpu.VMEM((H, B, DH), jnp.float32),
            pltpu.SemaphoreType.DMA((10,)), pltpu.SemaphoreType.DMA((NBUF, 2)),
        ],
        compiler_params=pltpu.CompilerParams(vmem_limit_bytes=100 * 1024 * 1024),
    )(A_x.reshape(B, D), A_k_cache, A_v_cache, A_wq, A_wo, B_w1.T, B_b1, B_w2, B_b2, c, w_mod)
    return out.reshape(B, Sq, D)
```

```python
import functools
import jax
import jax.numpy as jnp
from jax import lax
from jax.experimental import pallas as pl
from jax.experimental.pallas import tpu as pltpu

NBUF = 8
AHEAD = 4
CH = 128
_NT = (((1,), (1,)), ((), ()))


def _layernorm(x, eps=1e-5):
    m = jnp.mean(x, axis=-1, keepdims=True)
    d = x - m
    v = jnp.mean(d * d, axis=-1, keepdims=True)
    return d / jnp.sqrt(v + eps)


def _kernel(x_hbm, k_hbm, v_hbm, wq_hbm, wo_hbm, w1t_hbm, b1_hbm, w2_hbm, b2_hbm, c_hbm, wm_hbm,
            out_ref,
            x_v, c_v, b1_v, b2_v, wm_v, wq_v, wo_v, w1t_v, w2_v, kbuf, vbuf, q_s, mod_s, sem_s, sem_w, sem_kv):
    B, H, SK, DH = k_hbm.shape
    W = kbuf.shape[1]
    D = x_v.shape[1]
    F = w2_v.shape[0]
    NP = B * H
    NCH = W // CH
    f32, bf16 = jnp.float32, jnp.bfloat16
    cp = pltpu.make_async_copy

    def start_kv(p, j):
        h, b, slot = p // B, p % B, p % NBUF
        rows = pl.ds(SK - W + j * CH, CH)
        dst = pl.ds(j * CH, CH)
        if not isinstance(j, int):
            rows = pl.ds(pl.multiple_of(SK - W + j * CH, CH), CH)
            dst = pl.ds(pl.multiple_of(j * CH, CH), CH)
        cp(k_hbm.at[b, h, rows, :], kbuf.at[slot, dst], sem_kv.at[slot, 0]).start(priority=0)
        cp(v_hbm.at[b, h, rows, :], vbuf.at[slot, dst], sem_kv.at[slot, 1]).start(priority=1)

    def start_w(src, dst, sem, r0, nr, c0, nc, prio):
        if not isinstance(r0, int):
            r0 = pl.multiple_of(r0, 8)
        idx = (pl.ds(r0, nr), pl.ds(c0, nc))
        cp(src.at[idx], dst.at[idx], sem).start(priority=prio)

    def wait_all(dst, sem):
        cp(dst, dst, sem).wait()

    small = [cp(c_hbm, c_v, sem_s.at[0]), cp(x_hbm, x_v, sem_s.at[1]),
             cp(b1_hbm, b1_v, sem_s.at[2]), cp(b2_hbm, b2_v, sem_s.at[3])]
    for c_ in small:
        c_.start()

    @pl.loop(0, D // 8)
    def _(i):
        start_w(wm_hbm, wm_v, sem_w.at[0], i * 8, 8, 0, 3 * D, 0)
        start_w(wm_hbm, wm_v, sem_w.at[0], i * 8, 8, 3 * D, 3 * D, 1)

    @pl.loop(0, D // 8)
    def _(i):
        start_w(wq_hbm, wq_v, sem_w.at[1], i * 8, 8, 0, H * DH // 2, 0)
        start_w(wq_hbm, wq_v, sem_w.at[1], i * 8, 8, H * DH // 2, H * DH // 2, 1)

    for c_ in small:
        c_.wait()
    cc = c_v[...].astype(f32)
    sc = (cc * jax.nn.sigmoid(cc)).astype(bf16)
    x = x_v[...].astype(f32)
    ln = _layernorm(x)
    wait_all(wm_v, sem_w.at[0])
    mod_s[...] = jnp.dot(sc, wm_v[...], preferred_element_type=f32)
    h = (ln * (1.0 + mod_s[:, D:2 * D]) + mod_s[:, 0:D]).astype(bf16)

    half = H * DH // 2
    @pl.loop(0, half // 16)
    def _(i):
        start_w(wo_hbm, wo_v, sem_w.at[2], i * 16, 16, 0, D, 0)
        start_w(wo_hbm, wo_v, sem_w.at[2], half + i * 16, 16, 0, D, 1)

    wait_all(wq_v, sem_w.at[1])
    q = jnp.dot(h, wq_v[...], preferred_element_type=f32)
    for hh in range(H):
        q_s[hh] = q[:, hh * DH:(hh + 1) * DH]

    @pl.loop(0, AHEAD * NCH)
    def _(i):
        start_kv(i // NCH, i % NCH)

    wait_all(wo_v, sem_w.at[2])

    scale = DH ** -0.5
    row = lax.broadcasted_iota(jnp.int32, (B, DH), 0)
    NT = W // DH
    QK_ISSUE = (NCH * 5) // 8

    def attend(p, acc, issue):
        hh, b, slot = p // B, p % B, p % NBUF
        qh = q_s[hh].astype(bf16)
        wait_all(kbuf.at[slot], sem_kv.at[slot, 0])
        ss = []
        n = 0
        for j in range(NT):
            ss.append(lax.dot_general(qh, kbuf[slot, pl.ds(j * DH, DH), :], _NT, preferred_element_type=f32))
            while n < (j + 1) * QK_ISSUE // NT:
                issue(n)
                n += 1
        s = jnp.concatenate(ss, axis=-1) * scale
        m = jnp.max(s, axis=-1, keepdims=True)
        e = jnp.exp(s - m)
        l = jnp.sum(e, axis=-1, keepdims=True)
        e = e.astype(bf16)
        wait_all(vbuf.at[slot], sem_kv.at[slot, 1])
        o = jnp.zeros((B, DH), f32)
        for j in range(NT):
            o += jnp.dot(e[:, j * DH:(j + 1) * DH], vbuf[slot, pl.ds(j * DH, DH), :], preferred_element_type=f32)
            while n < QK_ISSUE + (j + 1) * (NCH - QK_ISSUE) // NT:
                issue(n)
                n += 1
        o = jnp.where(row == b, o / l, 0.0).astype(bf16)
        return acc + jnp.dot(o, wo_v[pl.ds(pl.multiple_of(hh * DH, DH), DH), :], preferred_element_type=f32)

    acc = lax.fori_loop(0, NP - AHEAD, lambda p, a: attend(p, a, lambda j: start_kv(p + AHEAD, j)),
                        jnp.zeros((B, D), f32))

    RW = 24
    NW = F // RW // 2
    PER = NW // AHEAD
    def issue_ffn(p, j):
        i = (p - (NP - AHEAD)) * PER + j
        if j < PER:
            start_w(w1t_hbm, w1t_v, sem_w.at[3], i * RW, RW, 0, D, 0)
            start_w(w1t_hbm, w1t_v, sem_w.at[3], F // 2 + i * RW, RW, 0, D, 1)
    acc = lax.fori_loop(NP - AHEAD, NP, lambda p, a: attend(p, a, lambda j: issue_ffn(p, j)), acc)

    @pl.loop(0, NW)
    def _(i):
        start_w(w2_hbm, w2_v, sem_w.at[4], i * RW, RW, 0, D, 0)
        start_w(w2_hbm, w2_v, sem_w.at[4], F // 2 + i * RW, RW, 0, D, 1)

    x1 = x + mod_s[:, 2 * D:3 * D] * acc
    h2 = (_layernorm(x1) * (1.0 + mod_s[:, 4 * D:5 * D]) + mod_s[:, 3 * D:4 * D]).astype(bf16)
    wait_all(w1t_v, sem_w.at[3])
    u = lax.dot_general(h2, w1t_v[...], _NT, preferred_element_type=f32) + b1_v[...].astype(f32)[None, :]
    g = jax.nn.gelu(u, approximate=True).astype(bf16)
    wait_all(w2_v, sem_w.at[4])
    y = jnp.dot(g, w2_v[...], preferred_element_type=f32) + b2_v[...].astype(f32)[None, :]
    out_ref[...] = (x1 + mod_s[:, 5 * D:6 * D] * y).astype(out_ref.dtype)


@jax.jit
def pallas_adaLN_cond__sliding_block_cached__dense_activation_gelu__decode_kernel(A_x, A_k_cache, A_v_cache, A_wq, A_wo, B_x, B_w1, B_b1, B_w2, B_b2, c, w_mod):
    del B_x
    B, Sq, D = A_x.shape
    _, H, SK, DH = A_k_cache.shape
    W = min(4096, max(256, SK // 4))
    F = B_w1.shape[1]
    bf16 = jnp.bfloat16
    hbm = pl.BlockSpec(memory_space=pltpu.HBM)
    out = pl.pallas_call(
        _kernel,
        in_specs=[hbm] * 11,
        out_specs=pl.BlockSpec(memory_space=pltpu.VMEM),
        out_shape=jax.ShapeDtypeStruct((B, D), A_x.dtype),
        scratch_shapes=[
            pltpu.VMEM((B, D), bf16), pltpu.VMEM((B, D), bf16),
            pltpu.VMEM((F,), bf16), pltpu.VMEM((D,), bf16),
            pltpu.VMEM((D, 6 * D), bf16), pltpu.VMEM((D, H * DH), bf16), pltpu.VMEM((H * DH, D), bf16),
            pltpu.VMEM((F, D), bf16), pltpu.VMEM((F, D), bf16),
            pltpu.VMEM((NBUF, W, DH), bf16), pltpu.VMEM((NBUF, W, DH), bf16),
            pltpu.VMEM((H, B, DH), jnp.float32), pltpu.VMEM((B, 6 * D), jnp.float32),
            pltpu.SemaphoreType.DMA((4,)), pltpu.SemaphoreType.DMA((5,)), pltpu.SemaphoreType.DMA((NBUF, 2)),
        ],
        compiler_params=pltpu.CompilerParams(vmem_limit_bytes=100 * 1024 * 1024, disable_bounds_checks=True),
    )(A_x.reshape(B, D), A_k_cache, A_v_cache, A_wq, A_wo, B_w1.T, B_b1, B_w2, B_b2, c, w_mod)
    return out.reshape(B, Sq, D)
```

```python
import jax
import jax.numpy as jnp
from jax import lax
from jax.experimental import pallas as pl
from jax.experimental.pallas import tpu as pltpu

_NBUF = 8
_AHEAD = 4
_KV_ROWS = 160
_W_ROWS = 32
_W2_GROUP_ENDS = (1408, 1664, 1728)
_CONTRACT_LAST = (((1,), (1,)), ((), ()))


def _layernorm(x, eps=1e-5):
    mean = jnp.mean(x, axis=-1, keepdims=True)
    centered = x - mean
    var = jnp.mean(centered * centered, axis=-1, keepdims=True)
    return centered / jnp.sqrt(var + eps)


def _kernel(
    x_hbm, k_hbm, v_hbm, wq_hbm, wo_hbm, w1t_hbm, b1_hbm, w2_hbm, b2_hbm, c_hbm, wmod_hbm,
    out_ref,
    x_v, c_v, b1_v, b2_v, wmod_v, wq_v, wo_v, w1t_v, w2_v, k_ring, v_ring, q_v, mod_v,
    sem_small, sem_w, sem_w2, sem_kv,
):
    B, H, SK, DH = k_hbm.shape
    W = k_ring.shape[1]
    F, D = w2_v.shape
    n_pairs = B * H
    n_tiles = W // DH
    kv_chunks = [(r, min(_KV_ROWS, W - r)) for r in range(0, W, _KV_ROWS)]
    f32, bf16 = jnp.float32, jnp.bfloat16
    copy = pltpu.make_async_copy

    def start_kv(pair, j):
        head, b, slot = pair // B, pair % B, pair % _NBUF
        r, n = kv_chunks[j]
        src, dst = pl.ds(SK - W + r, n), pl.ds(r, n)
        copy(k_hbm.at[b, head, src, :], k_ring.at[slot, dst], sem_kv.at[slot, 0]).start(priority=0)
        copy(v_hbm.at[b, head, src, :], v_ring.at[slot, dst], sem_kv.at[slot, 1]).start(priority=1)

    def start_block(src, dst, sem, row, n_rows, col, n_cols, priority):
        if not isinstance(row, int):
            row = pl.multiple_of(row, 8)
        idx = (pl.ds(row, n_rows), pl.ds(col, n_cols))
        copy(src.at[idx], dst.at[idx], sem).start(priority=priority)

    def wait_filled(buf, sem):
        copy(buf, buf, sem).wait()

    small = [
        copy(c_hbm, c_v, sem_small.at[0]),
        copy(x_hbm, x_v, sem_small.at[1]),
        copy(b1_hbm, b1_v, sem_small.at[2]),
        copy(b2_hbm, b2_v, sem_small.at[3]),
    ]
    for cp in small:
        cp.start()

    @pl.loop(0, D // 8)
    def _(i):
        start_block(wmod_hbm, wmod_v, sem_w.at[0], i * 8, 8, 0, 3 * D, 0)
        start_block(wmod_hbm, wmod_v, sem_w.at[0], i * 8, 8, 3 * D, 3 * D, 1)

    half = H * DH // 2

    @pl.loop(0, D // 8)
    def _(i):
        start_block(wq_hbm, wq_v, sem_w.at[1], i * 8, 8, 0, half, 0)
        start_block(wq_hbm, wq_v, sem_w.at[1], i * 8, 8, half, half, 1)

    for cp in small:
        cp.wait()
    c = c_v[...].astype(f32)
    x = x_v[...].astype(f32)
    wait_filled(wmod_v, sem_w.at[0])
    mod_v[...] = jnp.dot(
        (c * jax.nn.sigmoid(c)).astype(bf16), wmod_v[...], preferred_element_type=f32
    )

    def mod(i):
        return mod_v[:, i * D:(i + 1) * D]

    h = (_layernorm(x) * (1.0 + mod(1)) + mod(0)).astype(bf16)

    @pl.loop(0, half // _W_ROWS)
    def _(i):
        start_block(wo_hbm, wo_v, sem_w.at[2], i * _W_ROWS, _W_ROWS, 0, D, 0)
        start_block(wo_hbm, wo_v, sem_w.at[2], half + i * _W_ROWS, _W_ROWS, 0, D, 1)

    wait_filled(wq_v, sem_w.at[1])
    q = jnp.dot(h, wq_v[...], preferred_element_type=f32)
    for head in range(H):
        q_v[head] = q[:, head * DH:(head + 1) * DH]

    @pl.loop(0, _AHEAD)
    def _(pair):
        for j in range(len(kv_chunks)):
            start_kv(pair, j)

    wait_filled(wo_v, sem_w.at[2])

    batch_row = lax.broadcasted_iota(jnp.int32, (B, DH), 0)

    def attend(pair, acc, issue, n_issue):
        head, b, slot = pair // B, pair % B, pair % _NBUF
        n_qk = n_issue * 5 // 8
        issued = 0
        q_head = q_v[head].astype(bf16)
        wait_filled(k_ring.at[slot], sem_kv.at[slot, 0])
        scores = []
        for t in range(n_tiles):
            k_tile = k_ring[slot, pl.ds(t * DH, DH), :]
            scores.append(
                lax.dot_general(q_head, k_tile, _CONTRACT_LAST, preferred_element_type=f32)
            )
            while issued < (t + 1) * n_qk // n_tiles:
                issue(issued)
                issued += 1
        s = jnp.concatenate(scores, axis=-1) * DH ** -0.5
        e = jnp.exp(s - jnp.max(s, axis=-1, keepdims=True))
        denom = jnp.sum(e, axis=-1, keepdims=True)
        e = e.astype(bf16)
        wait_filled(v_ring.at[slot], sem_kv.at[slot, 1])
        o = jnp.zeros((B, DH), f32)
        for t in range(n_tiles):
            while issued < n_qk + t * (n_issue - n_qk) // (n_tiles - 1):
                issue(issued)
                issued += 1
            v_tile = v_ring[slot, pl.ds(t * DH, DH), :]
            o += jnp.dot(e[:, t * DH:(t + 1) * DH], v_tile, preferred_element_type=f32)
        assert issued == n_issue
        o = jnp.where(batch_row == b, o / denom, 0.0).astype(bf16)
        wo_head = wo_v[pl.ds(pl.multiple_of(head * DH, DH), DH), :]
        return acc + jnp.dot(o, wo_head, preferred_element_type=f32)

    n_main = n_pairs - _AHEAD
    attn = lax.fori_loop(
        0, n_main,
        lambda p, acc: attend(p, acc, lambda j: start_kv(p + _AHEAD, j), len(kv_chunks)),
        jnp.zeros((B, D), f32),
    )

    def start_mlp(i, group):
        start_block(w1t_hbm, w1t_v, sem_w.at[3], i * _W_ROWS, _W_ROWS, 0, D, 0)
        start_block(w2_hbm, w2_v, sem_w2.at[group], i * _W_ROWS, _W_ROWS, 0, D, 1)

    per_pair = min(_W2_GROUP_ENDS[0] // _W_ROWS // _AHEAD, len(kv_chunks))
    attn = lax.fori_loop(
        n_main, n_pairs,
        lambda p, acc: attend(p, acc, lambda j: start_mlp((p - n_main) * per_pair + j, 0), per_pair),
        attn,
    )
    for i in range(per_pair * _AHEAD, F // _W_ROWS):
        start_mlp(i, min(g for g, end in enumerate(_W2_GROUP_ENDS) if i * _W_ROWS < end))

    x = x + mod(2) * attn
    h = (_layernorm(x) * (1.0 + mod(4)) + mod(3)).astype(bf16)
    wait_filled(w1t_v, sem_w.at[3])
    u = lax.dot_general(h, w1t_v[...], _CONTRACT_LAST, preferred_element_type=f32)
    u = jax.nn.gelu(u + b1_v[...].astype(f32)[None, :], approximate=True).astype(bf16)
    y = b2_v[...].astype(f32)[None, :]
    begin = 0
    for g, end in enumerate(_W2_GROUP_ENDS):
        wait_filled(w2_v.at[pl.ds(begin, end - begin)], sem_w2.at[g])
        y = y + jnp.dot(u[:, begin:end], w2_v[begin:end, :], preferred_element_type=f32)
        begin = end
    out_ref[...] = (x + mod(5) * y).astype(out_ref.dtype)


@jax.jit
def pallas_adaLN_cond__sliding_block_cached__dense_activation_gelu__decode_kernel(
    A_x: jax.Array,
    A_k_cache: jax.Array,
    A_v_cache: jax.Array,
    A_wq: jax.Array,
    A_wo: jax.Array,
    B_x: jax.Array,
    B_w1: jax.Array,
    B_b1: jax.Array,
    B_w2: jax.Array,
    B_b2: jax.Array,
    c: jax.Array,
    w_mod: jax.Array,
):
    del B_x
    B, Sq, D = A_x.shape
    _, H, SK, DH = A_k_cache.shape
    W = min(4096, max(256, SK // 4))
    F = B_w1.shape[1]
    assert Sq == 1 and A_wq.shape == (D, H * DH) and W % DH == 0
    assert _W2_GROUP_ENDS[-1] == F and all(e % _W_ROWS == 0 for e in _W2_GROUP_ENDS)
    assert (H * DH // 2) % _W_ROWS == 0 and D % 128 == 0
    bf16, f32 = jnp.bfloat16, jnp.float32
    out = pl.pallas_call(
        _kernel,
        in_specs=[pl.BlockSpec(memory_space=pltpu.HBM)] * 11,
        out_specs=pl.BlockSpec(memory_space=pltpu.VMEM),
        out_shape=jax.ShapeDtypeStruct((B, D), A_x.dtype),
        scratch_shapes=[
            pltpu.VMEM((B, D), bf16),
            pltpu.VMEM((B, D), bf16),
            pltpu.VMEM((F,), bf16),
            pltpu.VMEM((D,), bf16),
            pltpu.VMEM((D, 6 * D), bf16),
            pltpu.VMEM((D, H * DH), bf16),
            pltpu.VMEM((H * DH, D), bf16),
            pltpu.VMEM((F, D), bf16),
            pltpu.VMEM((F, D), bf16),
            pltpu.VMEM((_NBUF, W, DH), bf16),
            pltpu.VMEM((_NBUF, W, DH), bf16),
            pltpu.VMEM((H, B, DH), f32),
            pltpu.VMEM((B, 6 * D), f32),
            pltpu.SemaphoreType.DMA((4,)),
            pltpu.SemaphoreType.DMA((4,)),
            pltpu.SemaphoreType.DMA((len(_W2_GROUP_ENDS),)),
            pltpu.SemaphoreType.DMA((_NBUF, 2)),
        ],
        compiler_params=pltpu.CompilerParams(vmem_limit_bytes=64 * 1024 * 1024),
    )(
        A_x.reshape(B, D), A_k_cache, A_v_cache, A_wq, A_wo, B_w1.T, B_b1, B_w2, B_b2, c, w_mod
    )
    return out.reshape(B, Sq, D)
```
